```python
import jax
import jax.numpy as jnp

def _softmax(x, axis=-1):
    return jax.nn.softmax(x, axis=axis)
def _gelu(x):
    return jax.nn.gelu(x, approximate=True)
def _silu(x):
    return jax.nn.silu(x)
def _sigmoid(x):
    return jax.nn.sigmoid(x)
def _layernorm(x, axis=-1, eps=1e-5):
    m = jnp.mean(x, axis=axis, keepdims=True)
    v = jnp.var(x, axis=axis, keepdims=True)
    return (x - m) / jnp.sqrt(v + eps)
def _scatter_add(tgt, idx, src, axis=0):
    return tgt.at[idx].add(src)
def _segment_sum(src, seg, n):
    return jax.ops.segment_sum(src, seg, n)
class _Rng:
    def __init__(self, key):
        self._k = key
    def _next(self):
        self._k, sub = jax.random.split(self._k)
        return sub
    def normal(self, shape):
        return jax.random.normal(self._next(), shape, dtype=jnp.bfloat16)
    def randint(self, lo, hi, shape):
        return jax.random.randint(self._next(), shape, lo, hi, dtype=jnp.int32)
    def uniform(self, shape, lo=0.0, hi=1.0):
        return jax.random.uniform(self._next(), shape, jnp.bfloat16, lo, hi)
    def permutation(self, n):
        return jax.random.permutation(self._next(), n)


kernel_name = 'recurrent_scan__sliding_block_cached__dense_activation_gelu__decode'

def setup_inputs():
    _rng = _Rng(jax.random.key(int.from_bytes(__import__("os").urandom(4), "little")))
    _w = (lambda a: (lambda t: t.astype(jnp.bfloat16) if jnp.issubdtype(t.dtype, jnp.floating) else t)(jnp.asarray(a)))
    def _A_setup():
        B, Sq, D = 2, 1, 576
        Hq, Hkv, Sk, Dh = 32, 16, 32768, 128
        assert Hq % Hkv == 0, (Hq, Hkv)
        return {
            "x": _w((lambda *s: _rng.normal(s) * 0.05)(B, Sq, D)),
            "k_cache": _w((lambda *s: _rng.normal(s) * 0.05)(B, Hkv, Sk, Dh)),
            "v_cache": _w((lambda *s: _rng.normal(s) * 0.05)(B, Hkv, Sk, Dh)),
            "wq": _w((lambda *s: _rng.normal(s) * 0.05)(D, Hq * Dh) * (D ** -0.5)),
            "wo": _w((lambda *s: _rng.normal(s) * 0.05)(Hq * Dh, D) * ((Hq * Dh) ** -0.5)),
        }
    _A_in = _A_setup()

    def _B_setup():
        B, S, D, F = 2, 1, 576, 4608
        return {
            "x": _w((lambda *s: _rng.normal(s) * 0.05)(B, S, D)),
            "w1": _w((lambda *s: _rng.normal(s) * 0.05)(D, F) * (D ** -0.5)),
            "b1": _w((lambda *s: _rng.normal(s) * 0.05)(F) * 0.01),
            "w2": _w((lambda *s: _rng.normal(s) * 0.05)(F, D) * (F ** -0.5)),
            "b2": _w((lambda *s: _rng.normal(s) * 0.05)(D) * 0.01),
        }
    _B_in = _B_setup()

    return {
        "A_x": _A_in["x"],
        "A_k_cache": _A_in["k_cache"],
        "A_v_cache": _A_in["v_cache"],
        "A_wq": _A_in["wq"],
        "A_wo": _A_in["wo"],
        "B_x": _B_in["x"],
        "B_w1": _B_in["w1"],
        "B_b1": _B_in["b1"],
        "B_w2": _B_in["w2"],
        "B_b2": _B_in["b2"],
    }

def reference(A_x, A_k_cache, A_v_cache, A_wq, A_wo, B_x, B_w1, B_b1, B_w2, B_b2):
    def _A_ref(x, k_cache, v_cache, wq, wo):
        B, Sq, D = x.shape
        Hq, Dh = 32, 128
        Hkv, Sk = k_cache.shape[1], k_cache.shape[2]
        W = min(4096, max(256, Sk // 4))
        rep = Hq // Hkv
        q = (lambda x, *d: x.transpose(*d))((x @ wq).reshape(B, Sq, Hq, Dh), 0, 2, 1, 3)
        k = jnp.repeat(k_cache[:, :, Sk - W:, :], rep, axis=1)
        v = jnp.repeat(v_cache[:, :, Sk - W:, :], rep, axis=1)
        scores = jnp.einsum("bhqd,bhkd->bhqk", q, k) * (Dh ** -0.5)
        p = _softmax(scores, axis=-1)
        o = jnp.einsum("bhqk,bhkd->bhqd", p, v)
        return (lambda x, *d: x.transpose(*d))(o, 0, 2, 1, 3).reshape(B, Sq, Hq * Dh) @ wo

    def _B_ref(x, w1, b1, w2, b2):
        h = jnp.einsum("bsd,df->bsf", x, w1) + b1
        h = _gelu(h)
        return jnp.einsum("bsf,fd->bsd", h, w2) + b2

    x = A_x
    xn = _layernorm(x, axis=-1)
    s = _A_ref(xn, A_k_cache, A_v_cache, A_wq, A_wo)
    g = _silu(_B_ref(xn, B_w1, B_b1, B_w2, B_b2))
    return x + s * g
```

```python
import functools

import jax
import jax.numpy as jnp
from jax import lax
import jax.experimental.pallas as pl
import jax.experimental.pallas.tpu as pltpu

B = 2
D = 576
HQ = 32
HKV = 16
DH = 128
SK = 32768
W = 4096
F = 4608
NPAIR = B * HKV
EPS = 1e-5
SCALE = DH ** -0.5

_NN = (((1,), (0,)), ((), ()))
_NT = (((1,), (1,)), ((), ()))

KV_DMA_ROWS = 512
KV_UNIT_ROWS = 1024
LOOKAHEAD = 8
W_DMA_ROWS = 16


def _row_groups(n, g):
    out = []
    r = 0
    while r < n:
        out.append((r, min(g, n - r)))
        r += g
    return out


def _kernel(x_hbm, k_hbm, v_hbm, wq_hbm, woT_hbm, w1_hbm, b1_hbm, w2T_hbm, b2_hbm,
            o_ref,
            kbuf, vbuf, wqb, wob, w1b, w2b, xb, b1b, b2b,
            qs, sc_s, p_s, o_s, acc_s,
            small_sems, w_sems, kv_sems):
    nu_half = W // KV_UNIT_ROWS
    nu = 2 * nu_half
    dma_per_unit = KV_UNIT_ROWS // KV_DMA_ROWS

    prio = [0]

    def next_prio():
        prio[0] ^= 1
        return prio[0]

    w_units = []
    for (r0, n) in _row_groups(D, 64):
        w_units.append((wq_hbm, wqb, r0, n))
    for (r0, n) in _row_groups(D, 64):
        w_units.append((w1_hbm, w1b, r0, n))
    for (r0, n) in _row_groups(D, 64):
        w_units.append((w2T_hbm, w2b, r0, n))
    for (r0, n) in _row_groups(D, 64):
        w_units.append((woT_hbm, wob, r0, n))
    n_static = len(w_units)

    def w_copies(i):
        src, dst, r0, n = w_units[i]
        return [pltpu.make_async_copy(src.at[pl.ds(r, m), :], dst.at[pl.ds(r, m), :], w_sems.at[i])
                for (r, m) in [(r0 + a, c) for (a, c) in _row_groups(n, W_DMA_ROWS)]]

    def kv_copies(p, j):
        h = p // 2
        b = p % 2
        src, dst = (k_hbm, kbuf) if j < nu_half else (v_hbm, vbuf)
        r0 = (j % nu_half) * KV_UNIT_ROWS
        out = []
        for c in range(dma_per_unit):
            r = r0 + c * KV_DMA_ROWS
            out.append(pltpu.make_async_copy(
                src.at[b, h, pl.ds(SK - W + r, KV_DMA_ROWS), :],
                dst.at[p, pl.ds(r, KV_DMA_ROWS), :],
                kv_sems.at[p * nu + j]))
        return out

    def start_unit(g):
        if g < n_static:
            for c in w_copies(g):
                c.start(priority=next_prio())
        else:
            p, j = divmod(g - n_static, nu)
            if p < NPAIR:
                for c in kv_copies(p, j):
                    c.start(priority=next_prio())

    def wait_w(i):
        for c in w_copies(i):
            c.wait()

    cx = pltpu.make_async_copy(x_hbm, xb, small_sems.at[0])
    cx.start()
    for g in range(LOOKAHEAD):
        start_unit(g)
    cb1 = pltpu.make_async_copy(b1_hbm, b1b, small_sems.at[1])
    cb1.start()
    cb2 = pltpu.make_async_copy(b2_hbm, b2b, small_sems.at[2])
    cb2.start()

    cx.wait()
    x = xb[...].astype(jnp.float32)
    mu = jnp.mean(x, axis=-1, keepdims=True)
    xc = x - mu
    var = jnp.mean(xc * xc, axis=-1, keepdims=True)
    xn = xc * lax.rsqrt(var + EPS)
    row_d = lax.broadcasted_iota(jnp.int32, (8, D), 0)
    xn8 = jnp.where((row_d & 2) == 0,
                    jnp.broadcast_to(xn[0:1], (8, D)),
                    jnp.broadcast_to(xn[1:2], (8, D))).astype(jnp.bfloat16)

    g = 0
    q_acc = None
    for (r0, n) in _row_groups(D, 64):
        wait_w(g)
        start_unit(g + LOOKAHEAD)
        part = lax.dot_general(xn8[:, r0:r0 + n], wqb[pl.ds(r0, n), :], _NN,
                               preferred_element_type=jnp.float32)
        q_acc = part if q_acc is None else q_acc + part
        g += 1
    row_h = lax.broadcasted_iota(jnp.int32, (8, DH), 0)
    odd = (row_h & 1) == 1
    for h in range(HKV):
        qs[h] = jnp.where(odd,
                          q_acc[:, (2 * h + 1) * DH:(2 * h + 2) * DH],
                          q_acc[:, (2 * h) * DH:(2 * h + 1) * DH])

    h_acc = None
    for (r0, n) in _row_groups(D, 64):
        wait_w(g)
        start_unit(g + LOOKAHEAD)
        part = lax.dot_general(xn8[:, r0:r0 + n], w1b[pl.ds(r0, n), :], _NN,
                               preferred_element_type=jnp.float32)
        h_acc = part if h_acc is None else h_acc + part
        g += 1
    cb1.wait()
    b1 = b1b[...].astype(jnp.float32).reshape(1, F)
    hh = jax.nn.gelu(h_acc + b1, approximate=True).astype(jnp.bfloat16)

    y_parts = []
    for (r0, n) in _row_groups(D, 64):
        wait_w(g)
        start_unit(g + LOOKAHEAD)
        y_parts.append(lax.dot_general(hh, w2b[pl.ds(r0, n), :], _NT,
                                       preferred_element_type=jnp.float32))
        g += 1
    cb2.wait()
    y = jnp.concatenate(y_parts, axis=1) + b2b[...].astype(jnp.float32).reshape(1, D)
    gate = jax.nn.silu(y)

    for (r0, n) in _row_groups(D, 64):
        wait_w(g)
        start_unit(g + LOOKAHEAD)
        g += 1

    acc_s[...] = jnp.zeros_like(acc_s)
    o_s[...] = jnp.zeros_like(o_s)

    def pair_body(p, carry):
        h = p // 2
        b = p % 2

        def step(j):
            for c in kv_copies(p, j):
                c.wait()
            jn = j + LOOKAHEAD
            dp, j2 = divmod(jn, nu)
            if dp == 0:
                for c in kv_copies(p, j2):
                    c.start(priority=next_prio())
            else:
                @pl.when(p + dp < NPAIR)
                def _():
                    for c in kv_copies(p + dp, j2):
                        c.start(priority=next_prio())

        q = qs[h].astype(jnp.bfloat16)
        for j in range(nu_half):
            step(j)
            r0 = j * KV_UNIT_ROWS
            sc_s[:, r0:r0 + KV_UNIT_ROWS] = lax.dot_general(
                q, kbuf[p, pl.ds(r0, KV_UNIT_ROWS), :], _NT,
                preferred_element_type=jnp.float32)
        sc = sc_s[...]
        m = jnp.max(sc, axis=-1, keepdims=True)
        e = jnp.exp((sc - m) * SCALE)
        l = jnp.sum(e, axis=-1, keepdims=True)
        p_s[...] = e.astype(jnp.bfloat16)
        o = None
        for j in range(nu_half):
            step(nu_half + j)
            r0 = j * KV_UNIT_ROWS
            part = lax.dot_general(p_s[:, r0:r0 + KV_UNIT_ROWS], vbuf[p, pl.ds(r0, KV_UNIT_ROWS), :], _NN,
                                   preferred_element_type=jnp.float32)
            o = part if o is None else o + part
        o = o / l
        mine = (row_h >> 1) == b
        o_new = jnp.where(mine, o, o_s[...])
        o_s[...] = o_new

        @pl.when(b == 1)
        def _():
            lhs = jnp.concatenate([jnp.where(odd, 0.0, o_new), jnp.where(odd, o_new, 0.0)],
                                  axis=1).astype(jnp.bfloat16)
            col = pl.multiple_of(h * (2 * DH), 2 * DH)
            acc_s[...] += lax.dot_general(lhs, wob[:, pl.ds(col, 2 * DH)], _NT,
                                          preferred_element_type=jnp.float32)
        return carry

    lax.fori_loop(0, NPAIR, pair_body, 0)

    acc = acc_s[...]
    s0 = acc[0:1] + acc[1:2]
    s1 = acc[2:3] + acc[3:4]
    s = jnp.concatenate([s0, s1], axis=0)
    gt = jnp.concatenate([gate[0:1], gate[2:3]], axis=0)
    o_ref[...] = (x + s * gt).astype(o_ref.dtype)


@jax.jit
def pallas_recurrent_scan__sliding_block_cached__dense_activation_gelu__decode_kernel(
    A_x: jax.Array,
    A_k_cache: jax.Array,
    A_v_cache: jax.Array,
    A_wq: jax.Array,
    A_wo: jax.Array,
    B_x: jax.Array,
    B_w1: jax.Array,
    B_b1: jax.Array,
    B_w2: jax.Array,
    B_b2: jax.Array,
):
    del B_x
    bf16 = jnp.bfloat16
    f32 = jnp.float32
    nu = 2 * (W // KV_UNIT_ROWS)
    n_static = 4 * len(_row_groups(D, 64))
    any_spec = pl.BlockSpec(memory_space=pl.ANY)
    out = pl.pallas_call(
        _kernel,
        out_shape=jax.ShapeDtypeStruct((B, D), bf16),
        in_specs=[any_spec] * 9,
        out_specs=pl.BlockSpec(memory_space=pltpu.VMEM),
        scratch_shapes=[
            pltpu.VMEM((NPAIR, W, DH), bf16),
            pltpu.VMEM((NPAIR, W, DH), bf16),
            pltpu.VMEM((D, HQ * DH), bf16),
            pltpu.VMEM((D, HQ * DH), bf16),
            pltpu.VMEM((D, F), bf16),
            pltpu.VMEM((D, F), bf16),
            pltpu.VMEM((B, D), bf16),
            pltpu.VMEM((F,), bf16),
            pltpu.VMEM((D,), bf16),
            pltpu.VMEM((HKV, 8, DH), f32),
            pltpu.VMEM((8, W), f32),
            pltpu.VMEM((8, W), bf16),
            pltpu.VMEM((8, DH), f32),
            pltpu.VMEM((8, D), f32),
            pltpu.SemaphoreType.DMA((3,)),
            pltpu.SemaphoreType.DMA((n_static,)),
            pltpu.SemaphoreType.DMA((NPAIR * nu,)),
        ],
        compiler_params=pltpu.CompilerParams(vmem_limit_bytes=110 * 1024 * 1024),
    )(A_x.reshape(B, D), A_k_cache, A_v_cache, A_wq, A_wo.T, B_w1, B_b1, B_w2.T, B_b2)
    return out.reshape(B, 1, D)
```

```python
import functools

import jax
import jax.numpy as jnp
from jax import lax
import jax.experimental.pallas as pl
import jax.experimental.pallas.tpu as pltpu

B = 2
D = 576
HQ = 32
HKV = 16
DH = 128
SK = 32768
W = 4096
F = 4608
EPS = 1e-5
SCALE = DH ** -0.5
_NN = (((1,), (0,)), ((), ()))
_NT = (((1,), (1,)), ((), ()))

SEG = W // 2
NSEG_ALL = SK // SEG
WR = D // 4
CR = 32
WC = 512
UR = 4
NU = SEG // CR // UR
LAST = HKV - 1
LA = 6
TAIL_V = (256,) * 8
TAIL_GROUPS = (4, 2, 1, 1)
N_TAIL_K = SEG // (2 * UR * CR)


def _kernel(x_hbm, k_hbm, v_hbm, wq_hbm, woT_hbm, w1_hbm, b1_hbm, w2T_hbm, b2_hbm,
            o_ref,
            kbuf, vbuf, wqb, wob, w1b, w2b, xb, b1b, b2b,
            qs, acc_s, gate_s,
            small_sems, w_sems, kv_sems, tail_sems):
    wpairs = [((wq_hbm, wqb), (w1_hbm, w1b)), ((w2T_hbm, w2b), (woT_hbm, wob))]
    n_wt = WR // 8

    def w_cols(ref, half):
        n = ref.shape[-1] // WC
        k = (n + 1) // 2
        return (0, k) if half == 0 else (k, n - k)

    def w_start(ph, t, half):
        sem = w_sems.at[(ph * n_wt + t) * 2 + half]
        seqs = []
        for (src, dst) in wpairs[ph]:
            c0, n = w_cols(src, half)
            seqs.append([pltpu.make_async_copy(src.at[i, :, pl.ds(8 * t, 8), pl.ds(c * WC, WC)],
                                               dst.at[i, :, pl.ds(8 * t, 8), pl.ds(c * WC, WC)], sem)
                         for c in range(c0, c0 + n) for i in range(2)])
        for n in range(max(len(seqs[0]), len(seqs[1]))):
            for th in range(2):
                if n < len(seqs[th]):
                    seqs[th][n].start(priority=th)

    def w_wait(ph, t, half):
        sem = w_sems.at[(ph * n_wt + t) * 2 + half]
        for (src, dst) in wpairs[ph]:
            c0, n = w_cols(src, half)
            v = dst.at[:, :, pl.ds(8 * t, 8), pl.ds(c0 * WC, n * WC)]
            pltpu.make_async_copy(v, v, sem).wait()

    def kv_copy(src, dst, p, b, r, n, sem):
        return pltpu.make_async_copy(src.at[b, p, pl.ds(NSEG_ALL - 2, 2), pl.ds(r, n), :],
                                     dst.at[p, b, :, pl.ds(r, n), :], sem)

    def kv_start(p, j):
        sem = kv_sems.at[(p % 2) * NU + j]
        for i in range(UR):
            r = (j * UR + i) * CR
            for b in range(B):
                kv_copy(k_hbm, kbuf, p, b, r, CR, sem).start(priority=0)
                kv_copy(v_hbm, vbuf, p, b, r, CR, sem).start(priority=1)

    def kv_wait(p, j):
        sem = kv_sems.at[(p % 2) * NU + j]
        for buf in (kbuf, vbuf):
            v = buf.at[p, :, :, pl.ds(j * UR * CR, UR * CR), :]
            pltpu.make_async_copy(v, v, sem).wait()

    tail_units = [(0, r, 2 * UR * CR) for r in range(0, SEG, 2 * UR * CR)]
    r_acc = 0
    for n in TAIL_V:
        tail_units.append((1, r_acc, n))
        r_acc += n
    n_tail = len(tail_units)

    def tail_start(j):
        is_v, r0, n = tail_units[j]
        src, dst = (v_hbm, vbuf) if is_v else (k_hbm, kbuf)
        for r in range(r0, r0 + n, CR):
            for b in range(B):
                kv_copy(src, dst, LAST, b, r, CR, tail_sems.at[j]).start(priority=b)

    def tail_wait(j):
        is_v, r0, n = tail_units[j]
        dst = vbuf if is_v else kbuf
        v = dst.at[LAST, :, :, pl.ds(r0, n), :]
        pltpu.make_async_copy(v, v, tail_sems.at[j]).wait()

    sunits = [("w", ph, t, half) for ph in range(2) for t in range(n_wt) for half in range(2)]
    n_w = len(sunits)
    sunits += [("kv", 0, j) for j in range(NU)] + [("kv", 1, j) for j in range(LA)]

    def s_start(g):
        u = sunits[g]
        if u[0] == "w":
            w_start(*u[1:])
        else:
            kv_start(u[1], u[2])

    def s_wait(g):
        u = sunits[g]
        if u[0] == "w":
            w_wait(*u[1:])
        else:
            kv_wait(u[1], u[2])

    cx = pltpu.make_async_copy(x_hbm, xb, small_sems.at[0])
    cb1 = pltpu.make_async_copy(b1_hbm, b1b, small_sems.at[1])
    cb2 = pltpu.make_async_copy(b2_hbm, b2b, small_sems.at[2])
    cx.start()
    for g in range(LA):
        s_start(g)
    cb1.start()
    cb2.start()

    cx.wait()
    x = xb[...].astype(jnp.float32)
    mu = jnp.mean(x, axis=-1, keepdims=True)
    xc = x - mu
    var = jnp.mean(xc * xc, axis=-1, keepdims=True)
    xn = xc * lax.rsqrt(var + EPS)
    row_d = lax.broadcasted_iota(jnp.int32, (8, D), 0)
    xn8 = jnp.where((row_d & 2) == 0,
                    jnp.broadcast_to(xn[0:1], (8, D)),
                    jnp.broadcast_to(xn[1:2], (8, D))).astype(jnp.bfloat16)
    row_h = lax.broadcasted_iota(jnp.int32, (8, DH), 0)
    odd = (row_h & 1) == 1

    st = {}

    def q_piece(c):
        wcols = wqb[:, :, :, pl.ds(c * 512, 512)].reshape(D, 512)
        q = lax.dot_general(xn8, wcols, _NN, preferred_element_type=jnp.float32)
        for hh in range(2):
            qs[2 * c + hh] = jnp.where(odd, q[:, (2 * hh + 1) * DH:(2 * hh + 2) * DH],
                                       q[:, (2 * hh) * DH:(2 * hh + 1) * DH])

    def h_piece(c):
        if c == 0:
            cb1.wait()
            st["b1"] = b1b[...].astype(jnp.float32).reshape(1, F)
            st["h"] = []
        wcols = w1b[:, :, :, pl.ds(c * 512, 512)].reshape(D, 512)
        pre = lax.dot_general(xn8, wcols, _NN, preferred_element_type=jnp.float32)
        st["h"].append(jax.nn.gelu(pre + st["b1"][:, c * 512:(c + 1) * 512],
                                   approximate=True).astype(jnp.bfloat16))

    def y_piece(i, kc):
        n = F // 4
        if i == 0 and kc == 0:
            st["hh"] = jnp.concatenate(st["h"], axis=1)
            st["y"] = [None] * 4
        part = lax.dot_general(st["hh"][:, kc * n:(kc + 1) * n], w2b[i // 2, i % 2, :, pl.ds(kc * n, n)], _NT,
                               preferred_element_type=jnp.float32)
        st["y"][i] = part if st["y"][i] is None else st["y"][i] + part
        if i == 3 and kc == 3:
            cb2.wait()
            y = jnp.concatenate(st["y"], axis=1) + b2b[...].astype(jnp.float32).reshape(1, D)
            gate_s[...] = jax.nn.silu(y)

    sched = {}
    pieces = [functools.partial(q_piece, c) for c in range(8)] + [functools.partial(h_piece, c) for c in range(9)]
    for n, pc in enumerate(pieces):
        sched[n_w // 2 + 2 * n] = pc
    for n in range(16):
        sched[n_w + n] = functools.partial(y_piece, n // 4, n % 4)
    for g in range(n_w + NU):
        s_wait(g)
        if g + LA < len(sunits):
            s_start(g + LA)
        if g in sched:
            sched[g]()
    acc_s[...] = jnp.zeros_like(acc_s)

    def wo_part(p, o0, o1):
        o = jnp.where(row_h < 2, o0, o1)
        lhs = jnp.concatenate([jnp.where(odd, 0.0, o), jnp.where(odd, o, 0.0)], axis=1).astype(jnp.bfloat16)
        col = p * (2 * DH)
        if not isinstance(p, int):
            col = pl.multiple_of(col, 2 * DH)
        wcols = wob[:, :, :, pl.ds(col, 2 * DH)].reshape(D, 2 * DH)
        return lax.dot_general(lhs, wcols, _NT, preferred_element_type=jnp.float32)

    def qk(a, p, b, s):
        if "q" not in a:
            a["q"] = qs[p].astype(jnp.bfloat16)
        a["sc", b, s] = lax.dot_general(a["q"], kbuf[p, b, s], _NT, preferred_element_type=jnp.float32)

    def sm(a, b):
        sc = jnp.concatenate([a["sc", b, 0], a["sc", b, 1]], axis=1)
        m = jnp.max(sc, axis=-1, keepdims=True)
        e = jnp.exp((sc - m) * SCALE)
        a["l", b] = jnp.sum(e, axis=-1, keepdims=True)
        a["p", b] = e.astype(jnp.bfloat16)

    def pv(a, p, b, s, r0=0, n=SEG):
        part = lax.dot_general(a["p", b][:, s * SEG + r0:s * SEG + r0 + n], vbuf[p, b, s, pl.ds(r0, n), :], _NN,
                               preferred_element_type=jnp.float32)
        a["o", b] = part if ("o", b) not in a else a["o", b] + part

    def wo(a, p):
        acc_s[...] += wo_part(p, a["o", 0] / a["l", 0], a["o", 1] / a["l", 1])

    def attend_pieces(a, p):
        out = []
        for b in range(B):
            out += [functools.partial(qk, a, p, b, 0), functools.partial(qk, a, p, b, 1),
                    functools.partial(sm, a, b),
                    functools.partial(pv, a, p, b, 0), functools.partial(pv, a, p, b, 1)]
        out.append(functools.partial(wo, a, p))
        return out

    def body(p, carry):
        pcs = attend_pieces({}, p)
        for j in range(NU):
            if j < len(pcs):
                pcs[j]()
            kv_wait(p + 1, j)
            jn = j + LA
            if jn < NU:
                kv_start(p + 1, jn)
            else:
                @pl.when(p + 2 < LAST)
                def _():
                    kv_start(p + 2, jn - NU)

                @pl.when(p + 2 == LAST)
                def _():
                    tail_start(jn - NU)
        return carry

    lax.fori_loop(0, LAST - 1, body, 0)

    pcs = attend_pieces({}, LAST - 1)
    for j in range(N_TAIL_K):
        pcs[j]()
        tail_wait(j)
        tail_start(j + LA)
    for pc in pcs[N_TAIL_K:]:
        pc()
    a = {}
    nxt = N_TAIL_K + LA
    for b in range(B):
        for s in range(2):
            qk(a, LAST, b, s)
            if nxt < n_tail:
                tail_start(nxt)
                nxt += 1
        sm(a, b)
    assert nxt == n_tail
    base_acc = acc_s[...]
    j = N_TAIL_K
    for g in TAIL_GROUPS:
        r0 = tail_units[j][1]
        n = 0
        for _ in range(g):
            tail_wait(j)
            n += tail_units[j][2]
            j += 1
        for b in range(B):
            for s in range(2):
                pv(a, LAST, b, s, r0, n)
    acc = base_acc + wo_part(LAST, a["o", 0] / a["l", 0], a["o", 1] / a["l", 1])
    s = jnp.concatenate([acc[0:1] + acc[1:2], acc[2:3] + acc[3:4]], axis=0)
    gate = gate_s[...]
    gt = jnp.concatenate([gate[0:1], gate[2:3]], axis=0)
    o_ref[...] = (x + s * gt).astype(o_ref.dtype)


@jax.jit
def pallas_recurrent_scan__sliding_block_cached__dense_activation_gelu__decode_kernel(
    A_x: jax.Array,
    A_k_cache: jax.Array,
    A_v_cache: jax.Array,
    A_wq: jax.Array,
    A_wo: jax.Array,
    B_x: jax.Array,
    B_w1: jax.Array,
    B_b1: jax.Array,
    B_w2: jax.Array,
    B_b2: jax.Array,
):
    del B_x
    bf16 = jnp.bfloat16
    f32 = jnp.float32
    any_spec = pl.BlockSpec(memory_space=pl.ANY)
    out = pl.pallas_call(
        _kernel,
        out_shape=jax.ShapeDtypeStruct((B, D), bf16),
        in_specs=[any_spec] * 9,
        out_specs=pl.BlockSpec(memory_space=pltpu.VMEM),
        scratch_shapes=[
            pltpu.VMEM((HKV, B, 2, SEG, DH), bf16),
            pltpu.VMEM((HKV, B, 2, SEG, DH), bf16),
            pltpu.VMEM((2, 2, WR, HQ * DH), bf16),
            pltpu.VMEM((2, 2, WR, HQ * DH), bf16),
            pltpu.VMEM((2, 2, WR, F), bf16),
            pltpu.VMEM((2, 2, WR, F), bf16),
            pltpu.VMEM((B, D), bf16),
            pltpu.VMEM((F,), bf16),
            pltpu.VMEM((D,), bf16),
            pltpu.VMEM((HKV, 8, DH), f32),
            pltpu.VMEM((8, D), f32),
            pltpu.VMEM((8, D), f32),
            pltpu.SemaphoreType.DMA((3,)),
            pltpu.SemaphoreType.DMA((2 * (WR // 8) * 2,)),
            pltpu.SemaphoreType.DMA((2 * NU,)),
            pltpu.SemaphoreType.DMA((N_TAIL_K + len(TAIL_V),)),
        ],
        compiler_params=pltpu.CompilerParams(
            vmem_limit_bytes=110 * 1024 * 1024,
            disable_bounds_checks=True,
            disable_semaphore_checks=True,
        ),
    )(A_x.reshape(B, D),
      A_k_cache.reshape(B, HKV, NSEG_ALL, SEG, DH), A_v_cache.reshape(B, HKV, NSEG_ALL, SEG, DH),
      A_wq.reshape(2, 2, WR, HQ * DH), A_wo.T.reshape(2, 2, WR, HQ * DH),
      B_w1.reshape(2, 2, WR, F), B_b1, B_w2.T.reshape(2, 2, WR, F), B_b2)
    return out.reshape(B, 1, D)
```

```python
import functools

import jax
import jax.numpy as jnp
from jax import lax
import jax.experimental.pallas as pl
import jax.experimental.pallas.tpu as pltpu

B = 2
D = 576
HQ = 32
HKV = 16
DH = 128
SK = 32768
W = 4096
F = 4608
EPS = 1e-5
SCALE = DH ** -0.5
_NN = (((1,), (0,)), ((), ()))
_NT = (((1,), (1,)), ((), ()))

SEG = W // 2
NSEG_ALL = SK // SEG
WR = D // 4
CR = 64
UR = 2
NU = SEG // CR // UR
LAST = HKV - 1
LA = 6
TAIL_V = (256,) * 8
TAIL_GROUPS = (4, 2, 1, 1)
N_TAIL_K = SEG // (2 * UR * CR)


def _kernel(x_hbm, k_hbm, v_hbm, wq_hbm, woT_hbm, w1_hbm, b1_hbm, w2T_hbm, b2_hbm,
            o_ref,
            kbuf, vbuf, wqb, wob, w1b, w2b, xb, b1b, b2b,
            qs, acc_s, gate_s,
            small_sems, w_sems, kv_sems, tail_sems):
    wpairs = [((wq_hbm, wqb), (w1_hbm, w1b)), ((w2T_hbm, w2b), (woT_hbm, wob))]
    n_wt = WR // 8

    def w_start(ph, t, half):
        sem = w_sems.at[(ph * n_wt + t) * 2 + half]
        seqs = []
        for (src, dst) in wpairs[ph]:
            cw = src.shape[-1] // 4
            seqs.append([pltpu.make_async_copy(src.at[i0, i1, pl.ds(8 * t, 8), pl.ds(c * cw, cw)],
                                               dst.at[i0, i1, pl.ds(8 * t, 8), pl.ds(c * cw, cw)], sem)
                         for c in range(2 * half, 2 * half + 2) for i1 in range(2) for i0 in range(2)])
        for n in range(len(seqs[0])):
            for th in range(2):
                seqs[th][n].start(priority=th)

    def w_wait(ph, t, half):
        sem = w_sems.at[(ph * n_wt + t) * 2 + half]
        for (src, dst) in wpairs[ph]:
            cw = src.shape[-1] // 2
            v = dst.at[:, :, pl.ds(8 * t, 8), pl.ds(half * cw, cw)]
            pltpu.make_async_copy(v, v, sem).wait()

    def kv_copy(src, dst, p, b, sg, r, n, sem):
        return pltpu.make_async_copy(src.at[b, p, NSEG_ALL - 2 + sg, pl.ds(r, n), :],
                                     dst.at[p, b, sg, pl.ds(r, n), :], sem)

    def kv_start(p, j):
        sem = kv_sems.at[(p % 2) * NU + j]
        for i in range(UR):
            r = (j * UR + i) * CR
            for sg in range(2):
                for (src, dst) in ((k_hbm, kbuf), (v_hbm, vbuf)):
                    for b in range(B):
                        kv_copy(src, dst, p, b, sg, r, CR, sem).start(priority=b)

    def kv_wait(p, j):
        sem = kv_sems.at[(p % 2) * NU + j]
        for buf in (kbuf, vbuf):
            v = buf.at[p, :, :, pl.ds(j * UR * CR, UR * CR), :]
            pltpu.make_async_copy(v, v, sem).wait()

    tail_units = [(0, r, 2 * UR * CR) for r in range(0, SEG, 2 * UR * CR)]
    r_acc = 0
    for n in TAIL_V:
        tail_units.append((1, r_acc, n))
        r_acc += n
    n_tail = len(tail_units)

    def tail_start(j):
        is_v, r0, n = tail_units[j]
        src, dst = (v_hbm, vbuf) if is_v else (k_hbm, kbuf)
        for r in range(r0, r0 + n, CR):
            for sg in range(2):
                for b in range(B):
                    kv_copy(src, dst, LAST, b, sg, r, CR, tail_sems.at[j]).start(priority=b)

    def tail_wait(j):
        is_v, r0, n = tail_units[j]
        dst = vbuf if is_v else kbuf
        v = dst.at[LAST, :, :, pl.ds(r0, n), :]
        pltpu.make_async_copy(v, v, tail_sems.at[j]).wait()

    sunits = [("w", ph, t, half) for ph in range(2) for t in range(n_wt) for half in range(2)]
    n_w = len(sunits)
    sunits += [("kv", 0, j) for j in range(NU)] + [("kv", 1, j) for j in range(LA)]

    def s_start(g):
        u = sunits[g]
        if u[0] == "w":
            w_start(*u[1:])
        else:
            kv_start(u[1], u[2])

    def s_wait(g):
        u = sunits[g]
        if u[0] == "w":
            w_wait(*u[1:])
        else:
            kv_wait(u[1], u[2])

    cx = pltpu.make_async_copy(x_hbm, xb, small_sems.at[0])
    cb1 = pltpu.make_async_copy(b1_hbm, b1b, small_sems.at[1])
    cb2 = pltpu.make_async_copy(b2_hbm, b2b, small_sems.at[2])
    cx.start()
    for g in range(LA):
        s_start(g)
    cb1.start()
    cb2.start()

    cx.wait()
    x = xb[...].astype(jnp.float32)
    mu = jnp.mean(x, axis=-1, keepdims=True)
    xc = x - mu
    var = jnp.mean(xc * xc, axis=-1, keepdims=True)
    xn = xc * lax.rsqrt(var + EPS)
    row_d = lax.broadcasted_iota(jnp.int32, (8, D), 0)
    xn8 = jnp.where((row_d & 2) == 0,
                    jnp.broadcast_to(xn[0:1], (8, D)),
                    jnp.broadcast_to(xn[1:2], (8, D))).astype(jnp.bfloat16)
    row_h = lax.broadcasted_iota(jnp.int32, (8, DH), 0)
    odd = (row_h & 1) == 1

    st = {}

    def q_piece(c):
        wcols = wqb[:, :, :, pl.ds(c * 512, 512)].reshape(D, 512)
        q = lax.dot_general(xn8, wcols, _NN, preferred_element_type=jnp.float32)
        for hh in range(2):
            qs[2 * c + hh] = jnp.where(odd, q[:, (2 * hh + 1) * DH:(2 * hh + 2) * DH],
                                       q[:, (2 * hh) * DH:(2 * hh + 1) * DH])

    def h_piece(c):
        if c == 0:
            cb1.wait()
            st["b1"] = b1b[...].astype(jnp.float32).reshape(1, F)
            st["h"] = []
        wcols = w1b[:, :, :, pl.ds(c * 512, 512)].reshape(D, 512)
        pre = lax.dot_general(xn8, wcols, _NN, preferred_element_type=jnp.float32)
        st["h"].append(jax.nn.gelu(pre + st["b1"][:, c * 512:(c + 1) * 512],
                                   approximate=True).astype(jnp.bfloat16))

    def y_piece(i, kc):
        n = F // 4
        if i == 0 and kc == 0:
            st["hh"] = jnp.concatenate(st["h"], axis=1)
            st["y"] = [None] * 4
        part = lax.dot_general(st["hh"][:, kc * n:(kc + 1) * n], w2b[i // 2, i % 2, :, pl.ds(kc * n, n)], _NT,
                               preferred_element_type=jnp.float32)
        st["y"][i] = part if st["y"][i] is None else st["y"][i] + part
        if i == 3 and kc == 3:
            cb2.wait()
            y = jnp.concatenate(st["y"], axis=1) + b2b[...].astype(jnp.float32).reshape(1, D)
            gate_s[...] = jax.nn.silu(y)

    sched = {}
    pieces = [functools.partial(q_piece, c) for c in range(8)] + [functools.partial(h_piece, c) for c in range(9)]
    for n, pc in enumerate(pieces):
        sched[n_w // 2 + 2 * n] = pc
    for n in range(16):
        sched[n_w + n] = functools.partial(y_piece, n // 4, n % 4)
    for g in range(n_w + NU):
        s_wait(g)
        if g + LA < len(sunits):
            s_start(g + LA)
        if g in sched:
            sched[g]()
    acc_s[...] = jnp.zeros_like(acc_s)

    def wo_part(p, o0, o1):
        o = jnp.where(row_h < 2, o0, o1)
        lhs = jnp.concatenate([jnp.where(odd, 0.0, o), jnp.where(odd, o, 0.0)], axis=1).astype(jnp.bfloat16)
        col = p * (2 * DH)
        if not isinstance(p, int):
            col = pl.multiple_of(col, 2 * DH)
        wcols = wob[:, :, :, pl.ds(col, 2 * DH)].reshape(D, 2 * DH)
        return lax.dot_general(lhs, wcols, _NT, preferred_element_type=jnp.float32)

    def qk(a, p, b, s):
        if "q" not in a:
            a["q"] = qs[p].astype(jnp.bfloat16)
        a["sc", b, s] = lax.dot_general(a["q"], kbuf[p, b, s], _NT, preferred_element_type=jnp.float32)

    def sm(a, b):
        sc = jnp.concatenate([a["sc", b, 0], a["sc", b, 1]], axis=1)
        m = jnp.max(sc, axis=-1, keepdims=True)
        e = jnp.exp((sc - m) * SCALE)
        a["l", b] = jnp.sum(e, axis=-1, keepdims=True)
        a["p", b] = e.astype(jnp.bfloat16)

    def pv(a, p, b, s, r0=0, n=SEG):
        part = lax.dot_general(a["p", b][:, s * SEG + r0:s * SEG + r0 + n], vbuf[p, b, s, pl.ds(r0, n), :], _NN,
                               preferred_element_type=jnp.float32)
        a["o", b] = part if ("o", b) not in a else a["o", b] + part

    def wo(a, p):
        acc_s[...] += wo_part(p, a["o", 0] / a["l", 0], a["o", 1] / a["l", 1])

    def attend_pieces(a, p):
        out = []
        for b in range(B):
            out += [functools.partial(qk, a, p, b, 0), functools.partial(qk, a, p, b, 1),
                    functools.partial(sm, a, b),
                    functools.partial(pv, a, p, b, 0), functools.partial(pv, a, p, b, 1)]
        out.append(functools.partial(wo, a, p))
        return out

    def body(p, carry):
        pcs = attend_pieces({}, p)
        for j in range(NU):
            if j < len(pcs):
                pcs[j]()
            kv_wait(p + 1, j)
            jn = j + LA
            if jn < NU:
                kv_start(p + 1, jn)
            else:
                @pl.when(p + 2 < LAST)
                def _():
                    kv_start(p + 2, jn - NU)

                @pl.when(p + 2 == LAST)
                def _():
                    tail_start(jn - NU)
        return carry

    lax.fori_loop(0, LAST - 1, body, 0)

    pcs = attend_pieces({}, LAST - 1)
    for j in range(N_TAIL_K):
        pcs[j]()
        tail_wait(j)
        tail_start(j + LA)
    for pc in pcs[N_TAIL_K:]:
        pc()
    a = {}
    nxt = N_TAIL_K + LA
    for b in range(B):
        for s in range(2):
            qk(a, LAST, b, s)
            if nxt < n_tail:
                tail_start(nxt)
                nxt += 1
        sm(a, b)
    assert nxt == n_tail
    base_acc = acc_s[...]
    j = N_TAIL_K
    for g in TAIL_GROUPS:
        r0 = tail_units[j][1]
        n = 0
        for _ in range(g):
            tail_wait(j)
            n += tail_units[j][2]
            j += 1
        for b in range(B):
            for s in range(2):
                pv(a, LAST, b, s, r0, n)
    acc = base_acc + wo_part(LAST, a["o", 0] / a["l", 0], a["o", 1] / a["l", 1])
    s = jnp.concatenate([acc[0:1] + acc[1:2], acc[2:3] + acc[3:4]], axis=0)
    gate = gate_s[...]
    gt = jnp.concatenate([gate[0:1], gate[2:3]], axis=0)
    o_ref[...] = (x + s * gt).astype(o_ref.dtype)


@jax.jit
def pallas_recurrent_scan__sliding_block_cached__dense_activation_gelu__decode_kernel(
    A_x: jax.Array,
    A_k_cache: jax.Array,
    A_v_cache: jax.Array,
    A_wq: jax.Array,
    A_wo: jax.Array,
    B_x: jax.Array,
    B_w1: jax.Array,
    B_b1: jax.Array,
    B_w2: jax.Array,
    B_b2: jax.Array,
):
    del B_x
    bf16 = jnp.bfloat16
    f32 = jnp.float32
    any_spec = pl.BlockSpec(memory_space=pl.ANY)
    out = pl.pallas_call(
        _kernel,
        out_shape=jax.ShapeDtypeStruct((B, D), bf16),
        in_specs=[any_spec] * 9,
        out_specs=pl.BlockSpec(memory_space=pltpu.VMEM),
        scratch_shapes=[
            pltpu.VMEM((HKV, B, 2, SEG, DH), bf16),
            pltpu.VMEM((HKV, B, 2, SEG, DH), bf16),
            pltpu.VMEM((2, 2, WR, HQ * DH), bf16),
            pltpu.VMEM((2, 2, WR, HQ * DH), bf16),
            pltpu.VMEM((2, 2, WR, F), bf16),
            pltpu.VMEM((2, 2, WR, F), bf16),
            pltpu.VMEM((B, D), bf16),
            pltpu.VMEM((F,), bf16),
            pltpu.VMEM((D,), bf16),
            pltpu.VMEM((HKV, 8, DH), f32),
            pltpu.VMEM((8, D), f32),
            pltpu.VMEM((8, D), f32),
            pltpu.SemaphoreType.DMA((3,)),
            pltpu.SemaphoreType.DMA((2 * (WR // 8) * 2,)),
            pltpu.SemaphoreType.DMA((2 * NU,)),
            pltpu.SemaphoreType.DMA((N_TAIL_K + len(TAIL_V),)),
        ],
        compiler_params=pltpu.CompilerParams(
            vmem_limit_bytes=110 * 1024 * 1024,
            disable_bounds_checks=True,
            disable_semaphore_checks=True,
        ),
    )(A_x.reshape(B, D),
      A_k_cache.reshape(B, HKV, NSEG_ALL, SEG, DH), A_v_cache.reshape(B, HKV, NSEG_ALL, SEG, DH),
      A_wq.reshape(2, 2, WR, HQ * DH), A_wo.T.reshape(2, 2, WR, HQ * DH),
      B_w1.reshape(2, 2, WR, F), B_b1, B_w2.T.reshape(2, 2, WR, F), B_b2)
    return out.reshape(B, 1, D)
```

```python
import functools

import jax
import jax.numpy as jnp
from jax import lax
import jax.experimental.pallas as pl
import jax.experimental.pallas.tpu as pltpu

B = 2
D = 576
HQ = 32
HKV = 16
DH = 128
SK = 32768
W = 4096
F = 4608
EPS = 1e-5
SCALE = DH ** -0.5
_NN = (((1,), (0,)), ((), ()))
_NT = (((1,), (1,)), ((), ()))

SEG = W // 2
NSEG_ALL = SK // SEG
WR = D // 4
N_WT = WR // 8
CR = 64
UROWS = 2 * CR
NU = SEG // UROWS
LAST = HKV - 1
LA = 6
TROWS = 2 * UROWS
N_TAIL_K = SEG // TROWS
N_TAIL = 2 * N_TAIL_K
TAIL_GROUPS = (4, 2, 1, 1)
TAIL_PIECES = (1, 2, 1, 2, 1, 1, 2, 1)


def _kernel(x_hbm, k_hbm, v_hbm, wq_hbm, woT_hbm, w1_hbm, b1_hbm, w2T_hbm, b2_hbm,
            o_ref,
            kbuf, vbuf, wqb, wob, w1b, w2b, xb, b1b, b2b,
            qs, acc_s, gate_s,
            small_sems, w_sems, kv_sems, tail_sems):
    wpairs = [((wq_hbm, wqb), (w1_hbm, w1b)), ((w2T_hbm, w2b), (woT_hbm, wob))]

    def w_sem(ph, t, half, m):
        return w_sems.at[((ph * N_WT + t) * 2 + half) * 2 + m]

    def w_start(ph, t, half):
        for c in range(2 * half, 2 * half + 2):
            for i1 in range(2):
                for i0 in range(2):
                    for m, (src, dst) in enumerate(wpairs[ph]):
                        cw = src.shape[-1] // 4
                        pltpu.make_async_copy(src.at[i0, i1, pl.ds(8 * t, 8), pl.ds(c * cw, cw)],
                                              dst.at[i0, i1, pl.ds(8 * t, 8), pl.ds(c * cw, cw)],
                                              w_sem(ph, t, half, m)).start(priority=m)

    def w_wait(ph, t, half):
        for m, (_, dst) in enumerate(wpairs[ph]):
            cw = dst.shape[-1] // 2
            v = dst.at[:, :, pl.ds(8 * t, 8), pl.ds(half * cw, cw)]
            pltpu.make_async_copy(v, v, w_sem(ph, t, half, m)).wait()

    def kv_copy(src, dst, p, b, sg, r, sem):
        return pltpu.make_async_copy(src.at[b, p, NSEG_ALL - 2 + sg, pl.ds(r, CR), :],
                                     dst.at[p, b, sg, pl.ds(r, CR), :], sem)

    def kv_sem(p, j, kv):
        return kv_sems.at[((p % 2) * NU + j) * 2 + kv]

    def kv_start(p, j):
        for r in range(j * UROWS, (j + 1) * UROWS, CR):
            for sg in range(2):
                for kv, (src, dst) in enumerate(((k_hbm, kbuf), (v_hbm, vbuf))):
                    for b in range(B):
                        kv_copy(src, dst, p, b, sg, r, kv_sem(p, j, kv)).start(priority=b)

    def kv_wait(p, j):
        for kv, buf in enumerate((kbuf, vbuf)):
            v = buf.at[p, :, :, pl.ds(j * UROWS, UROWS), :]
            pltpu.make_async_copy(v, v, kv_sem(p, j, kv)).wait()

    def tail_start(j):
        src, dst = (k_hbm, kbuf) if j < N_TAIL_K else (v_hbm, vbuf)
        r0 = (j % N_TAIL_K) * TROWS
        for r in range(r0, r0 + TROWS, CR):
            for sg in range(2):
                for b in range(B):
                    kv_copy(src, dst, LAST, b, sg, r, tail_sems.at[j]).start(priority=b)

    def tail_wait(j):
        dst = kbuf if j < N_TAIL_K else vbuf
        v = dst.at[LAST, :, :, pl.ds((j % N_TAIL_K) * TROWS, TROWS), :]
        pltpu.make_async_copy(v, v, tail_sems.at[j]).wait()

    sunits = [("w", ph, t, half) for ph in range(2) for t in range(N_WT) for half in range(2)]
    n_w = len(sunits)
    sunits += [("kv", 0, j) for j in range(NU)] + [("kv", 1, j) for j in range(LA)]

    def s_start(g):
        u = sunits[g]
        if u[0] == "w":
            w_start(*u[1:])
        else:
            kv_start(u[1], u[2])

    def s_wait(g):
        u = sunits[g]
        if u[0] == "w":
            w_wait(*u[1:])
        else:
            kv_wait(u[1], u[2])

    cx = pltpu.make_async_copy(x_hbm, xb, small_sems.at[0])
    cb1 = pltpu.make_async_copy(b1_hbm, b1b, small_sems.at[1])
    cb2 = pltpu.make_async_copy(b2_hbm, b2b, small_sems.at[2])
    cx.start()
    for g in range(LA):
        s_start(g)
    cb1.start()
    cb2.start()

    cx.wait()
    x = xb[...].astype(jnp.float32)
    mu = jnp.mean(x, axis=-1, keepdims=True)
    xc = x - mu
    var = jnp.mean(xc * xc, axis=-1, keepdims=True)
    xn = xc * lax.rsqrt(var + EPS)
    row_d = lax.broadcasted_iota(jnp.int32, (8, D), 0)
    xn8 = jnp.where((row_d & 2) == 0,
                    jnp.broadcast_to(xn[0:1], (8, D)),
                    jnp.broadcast_to(xn[1:2], (8, D))).astype(jnp.bfloat16)
    row_h = lax.broadcasted_iota(jnp.int32, (8, DH), 0)
    odd = (row_h & 1) == 1

    st = {}

    def q_piece(c):
        wcols = wqb[:, :, :, pl.ds(c * 512, 512)].reshape(D, 512)
        q = lax.dot_general(xn8, wcols, _NN, preferred_element_type=jnp.float32)
        for hh in range(2):
            qs[2 * c + hh] = jnp.where(odd, q[:, (2 * hh + 1) * DH:(2 * hh + 2) * DH],
                                       q[:, (2 * hh) * DH:(2 * hh + 1) * DH])

    def h_piece(c):
        if c == 0:
            cb1.wait()
            st["b1"] = b1b[...].astype(jnp.float32).reshape(1, F)
            st["h"] = []
        wcols = w1b[:, :, :, pl.ds(c * 512, 512)].reshape(D, 512)
        pre = lax.dot_general(xn8, wcols, _NN, preferred_element_type=jnp.float32)
        st["h"].append(jax.nn.gelu(pre + st["b1"][:, c * 512:(c + 1) * 512],
                                   approximate=True).astype(jnp.bfloat16))

    def y_piece(i, kc):
        n = F // 4
        if i == 0 and kc == 0:
            st["hh"] = jnp.concatenate(st["h"], axis=1)
            st["y"] = [None] * 4
        part = lax.dot_general(st["hh"][:, kc * n:(kc + 1) * n], w2b[i // 2, i % 2, :, pl.ds(kc * n, n)], _NT,
                               preferred_element_type=jnp.float32)
        st["y"][i] = part if st["y"][i] is None else st["y"][i] + part

    def y_fin():
        cb2.wait()
        y = jnp.concatenate(st["y"], axis=1) + b2b[...].astype(jnp.float32).reshape(1, D)
        gate_s[...] = jax.nn.silu(y)
        acc_s[...] = jnp.zeros_like(acc_s)

    sched = {}
    pieces = [functools.partial(q_piece, c) for c in range(8)] + [functools.partial(h_piece, c) for c in range(9)]
    for n, pc in enumerate(pieces):
        sched[n_w // 2 + 2 * n] = pc
    pieces = [functools.partial(y_piece, n // 4, n % 4) for n in range(16)] + [y_fin]
    for n, pc in enumerate(pieces):
        sched[n_w - 1 + n] = pc
    for g in range(n_w + NU):
        s_wait(g)
        if g + LA < len(sunits):
            s_start(g + LA)
        if g in sched:
            sched[g]()

    def wo_part(p, o0, o1):
        o = jnp.where(row_h < 2, o0, o1)
        lhs = jnp.concatenate([jnp.where(odd, 0.0, o), jnp.where(odd, o, 0.0)], axis=1).astype(jnp.bfloat16)
        col = p * (2 * DH)
        if not isinstance(p, int):
            col = pl.multiple_of(col, 2 * DH)
        wcols = wob[:, :, :, pl.ds(col, 2 * DH)].reshape(D, 2 * DH)
        return lax.dot_general(lhs, wcols, _NT, preferred_element_type=jnp.float32)

    def qk(a, p, b, s):
        if "q" not in a:
            a["q"] = qs[p].astype(jnp.bfloat16)
        a["sc", b, s] = lax.dot_general(a["q"], kbuf[p, b, s], _NT, preferred_element_type=jnp.float32)

    def sm(a, b):
        sc = jnp.concatenate([a["sc", b, 0], a["sc", b, 1]], axis=1)
        m = jnp.max(sc, axis=-1, keepdims=True)
        e = jnp.exp((sc - m) * SCALE)
        a["rl", b] = 1.0 / jnp.sum(e, axis=-1, keepdims=True)
        a["p", b] = e.astype(jnp.bfloat16)

    def pv(a, p, b, s, r0=0, n=SEG):
        part = lax.dot_general(a["p", b][:, s * SEG + r0:s * SEG + r0 + n], vbuf[p, b, s, pl.ds(r0, n), :], _NN,
                               preferred_element_type=jnp.float32)
        a["o", b] = part if ("o", b) not in a else a["o", b] + part

    def wo(a, p):
        acc_s[...] += wo_part(p, a["o", 0] * a["rl", 0], a["o", 1] * a["rl", 1])

    def attend_pieces(a, p):
        out = []
        for b in range(B):
            out += [functools.partial(qk, a, p, b, 0), functools.partial(qk, a, p, b, 1),
                    functools.partial(sm, a, b),
                    functools.partial(pv, a, p, b, 0), functools.partial(pv, a, p, b, 1)]
        out.append(functools.partial(wo, a, p))
        return out

    def body(p, carry):
        pcs = attend_pieces({}, p)
        for j in range(NU):
            kv_wait(p + 1, j)
            jn = j + LA
            if jn < NU:
                kv_start(p + 1, jn)
            else:
                @pl.when(p + 2 < LAST)
                def _():
                    kv_start(p + 2, jn - NU)

                @pl.when(p + 2 == LAST)
                def _():
                    tail_start(jn - NU)
            if j < len(pcs):
                pcs[j]()
        return carry

    lax.fori_loop(0, LAST - 1, body, 0)

    pcs = attend_pieces({}, LAST - 1)
    nxt = LA
    for j in range(N_TAIL_K):
        tail_wait(j)
        tail_start(nxt)
        nxt += 1
        for _ in range(TAIL_PIECES[j]):
            pcs.pop(0)()
    assert not pcs
    a = {}
    waited = N_TAIL_K
    pcs = []
    for b in range(B):
        pcs += [functools.partial(qk, a, LAST, b, 0), functools.partial(qk, a, LAST, b, 1),
                functools.partial(sm, a, b)]
    for pc in pcs:
        pc()
        if nxt < N_TAIL:
            tail_wait(waited)
            waited += 1
            tail_start(nxt)
            nxt += 1
    assert nxt == N_TAIL
    j = N_TAIL_K
    for g in TAIL_GROUPS:
        r0 = (j - N_TAIL_K) * TROWS
        for _ in range(g):
            if j >= waited:
                tail_wait(j)
                waited = j + 1
            j += 1
        for b in range(B):
            for s in range(2):
                pv(a, LAST, b, s, r0, g * TROWS)
    assert j == N_TAIL and waited == N_TAIL
    acc = acc_s[...] + wo_part(LAST, a["o", 0] * a["rl", 0], a["o", 1] * a["rl", 1])
    s = jnp.concatenate([acc[0:1] + acc[1:2], acc[2:3] + acc[3:4]], axis=0)
    gate = gate_s[...]
    gt = jnp.concatenate([gate[0:1], gate[2:3]], axis=0)
    o_ref[...] = (x + s * gt).astype(o_ref.dtype)


def _call(x2, k5, v5, wq4, woT4, w14, b1, w2T4, b2, **kw):
    bf16 = jnp.bfloat16
    f32 = jnp.float32
    any_spec = pl.BlockSpec(memory_space=pl.ANY)
    return pl.pallas_call(
        _kernel,
        out_shape=jax.ShapeDtypeStruct((B, D), bf16),
        in_specs=[any_spec] * 9,
        out_specs=pl.BlockSpec(memory_space=pltpu.VMEM),
        scratch_shapes=[
            pltpu.VMEM((HKV, B, 2, SEG, DH), bf16),
            pltpu.VMEM((HKV, B, 2, SEG, DH), bf16),
            pltpu.VMEM((2, 2, WR, HQ * DH), bf16),
            pltpu.VMEM((2, 2, WR, HQ * DH), bf16),
            pltpu.VMEM((2, 2, WR, F), bf16),
            pltpu.VMEM((2, 2, WR, F), bf16),
            pltpu.VMEM((B, D), bf16),
            pltpu.VMEM((F,), bf16),
            pltpu.VMEM((D,), bf16),
            pltpu.VMEM((HKV, 8, DH), f32),
            pltpu.VMEM((8, D), f32),
            pltpu.VMEM((8, D), f32),
            pltpu.SemaphoreType.DMA((3,)),
            pltpu.SemaphoreType.DMA((2 * N_WT * 2 * 2,)),
            pltpu.SemaphoreType.DMA((2 * NU * 2,)),
            pltpu.SemaphoreType.DMA((N_TAIL,)),
        ],
        compiler_params=pltpu.CompilerParams(
            vmem_limit_bytes=110 * 1024 * 1024,
            disable_bounds_checks=True,
            disable_semaphore_checks=True,
        ),
        **kw,
    )(x2, k5, v5, wq4, woT4, w14, b1, w2T4, b2)


@jax.jit
def pallas_recurrent_scan__sliding_block_cached__dense_activation_gelu__decode_kernel(
    A_x: jax.Array,
    A_k_cache: jax.Array,
    A_v_cache: jax.Array,
    A_wq: jax.Array,
    A_wo: jax.Array,
    B_x: jax.Array,
    B_w1: jax.Array,
    B_b1: jax.Array,
    B_w2: jax.Array,
    B_b2: jax.Array,
):
    del B_x
    out = _call(A_x.reshape(B, D),
                A_k_cache.reshape(B, HKV, NSEG_ALL, SEG, DH), A_v_cache.reshape(B, HKV, NSEG_ALL, SEG, DH),
                A_wq.reshape(2, 2, WR, HQ * DH), A_wo.T.reshape(2, 2, WR, HQ * DH),
                B_w1.reshape(2, 2, WR, F), B_b1, B_w2.T.reshape(2, 2, WR, F), B_b2)
    return out.reshape(B, 1, D)
```
